```python
import os as _os
_os.environ.setdefault("JAX_PLATFORMS", "cpu")
import jax
import jax.numpy as jnp

def _softmax(x, axis=-1):
    return jax.nn.softmax(x, axis=axis)
def _gelu(x):
    return jax.nn.gelu(x, approximate=True)
def _silu(x):
    return jax.nn.silu(x)
def _sigmoid(x):
    return jax.nn.sigmoid(x)
def _layernorm(x, axis=-1, eps=1e-5):
    m = jnp.mean(x, axis=axis, keepdims=True)
    v = jnp.var(x, axis=axis, keepdims=True)
    return (x - m) / jnp.sqrt(v + eps)
def _scatter_add(tgt, idx, src, axis=0):
    return tgt.at[idx].add(src)
def _segment_sum(src, seg, n):
    return jax.ops.segment_sum(src, seg, n)
class _Rng:
    def __init__(self, key):
        self._k = key
    def _next(self):
        self._k, sub = jax.random.split(self._k)
        return sub
    def normal(self, shape):
        return jax.random.normal(self._next(), shape, dtype=jnp.bfloat16)
    def randint(self, lo, hi, shape):
        return jax.random.randint(self._next(), shape, lo, hi, dtype=jnp.int32)
    def uniform(self, shape, lo=0.0, hi=1.0):
        return jax.random.uniform(self._next(), shape, jnp.bfloat16, lo, hi)
    def permutation(self, n):
        return jax.random.permutation(self._next(), n)


kernel_name = 'standalone__mha_softmax__near_ridge'

def setup_inputs():
    _rng = _Rng(jax.random.key(int.from_bytes(__import__("os").urandom(4), "little")))
    _w = (lambda a: (lambda t: t.astype(jnp.bfloat16) if jnp.issubdtype(t.dtype, jnp.floating) else t)(jnp.asarray(a)))
    B, H, Sq, Sk, D = 8, 16, 192, 1024, 256
    return {
        "q": _w((lambda *s: _rng.normal(s) * 0.4)(B, H, Sq, D)),
        "k": _w((lambda *s: _rng.normal(s) * 0.4)(B, H, Sk, D)),
        "v": _w((lambda *s: _rng.normal(s) * 0.05)(B, H, Sk, D)),
    }

def reference(q, k, v):
    scale = q.shape[-1] ** -0.5
    scores = jnp.einsum("bhqd,bhkd->bhqk", q, k) * scale
    p = _softmax(scores, axis=-1)
    return jnp.einsum("bhqk,bhkd->bhqd", p, v)
```

```python
import functools
import math

import jax
import jax.numpy as jnp
import jax.experimental.pallas as pl
import jax.experimental.pallas.tpu as pltpu


def _attn_kernel(q_ref, k_ref, v_ref, o_ref, *, scale):
    q = q_ref[0]
    k = k_ref[0]
    v = v_ref[0]
    s = jax.lax.dot_general(
        q, k, (((1,), (1,)), ((), ())), preferred_element_type=jnp.float32
    )
    m = jnp.max(s, axis=-1, keepdims=True)
    p = jnp.exp((s - m) * scale)
    l = jnp.sum(p, axis=-1, keepdims=True)
    o = jnp.dot(p.astype(jnp.bfloat16), v, preferred_element_type=jnp.float32)
    o_ref[0] = (o / l).astype(o_ref.dtype)


@jax.jit
def pallas_standalone__mha_softmax__near_ridge_kernel(
    q: jax.Array,
    k: jax.Array,
    v: jax.Array,
):
    B, H, Sq, D = q.shape
    Sk = k.shape[2]
    BH = B * H
    scale = float(D) ** -0.5
    q3 = q.reshape(BH, Sq, D)
    k3 = k.reshape(BH, Sk, D)
    v3 = v.reshape(BH, Sk, D)
    out = pl.pallas_call(
        functools.partial(_attn_kernel, scale=scale),
        grid=(BH,),
        in_specs=[
            pl.BlockSpec((1, Sq, D), lambda i: (i, 0, 0)),
            pl.BlockSpec((1, Sk, D), lambda i: (i, 0, 0)),
            pl.BlockSpec((1, Sk, D), lambda i: (i, 0, 0)),
        ],
        out_specs=pl.BlockSpec((1, Sq, D), lambda i: (i, 0, 0)),
        out_shape=jax.ShapeDtypeStruct((BH, Sq, D), q.dtype),
        compiler_params=pltpu.CompilerParams(
            dimension_semantics=("parallel",),
            vmem_limit_bytes=64 * 1024 * 1024,
        ),
    )(q3, k3, v3)
    return out.reshape(B, H, Sq, D)
```

```python
import functools

import jax
import jax.numpy as jnp
import jax.experimental.pallas as pl
import jax.experimental.pallas.tpu as pltpu

_NBUF = 3
_V_SPLIT = 256
_W_ROWS = 32


def _attention_head(q, k, v, scale):
    s = jax.lax.dot_general(
        q, k, (((1,), (1,)), ((), ())), preferred_element_type=jnp.float32
    )
    m = jnp.max(s, axis=-1, keepdims=True)
    p = jnp.exp((s - m) * scale)
    l = jnp.sum(p, axis=-1, keepdims=True)
    o = jnp.dot(p.astype(v.dtype), v, preferred_element_type=jnp.float32)
    return o / l


def _kernel(q_hbm, k_hbm, v_hbm, o_hbm, qbuf, kbuf, vbuf, obuf, sems, osem, *, scale):
    B, H, Sk, _ = k_hbm.shape
    Sq = q_hbm.shape[2]
    n = B * H
    vs = _V_SPLIT

    def early_copies(i):
        h, b, slot = i // B, i % B, i % _NBUF
        return [
            pltpu.make_async_copy(q_hbm.at[b, h], qbuf.at[slot], sems.at[0, slot]),
            pltpu.make_async_copy(k_hbm.at[b, h], kbuf.at[slot], sems.at[1, slot]),
            pltpu.make_async_copy(
                v_hbm.at[b, h, pl.ds(0, vs)],
                vbuf.at[slot, pl.ds(0, vs)],
                sems.at[2, slot],
            ),
        ]

    def late_copy(i):
        h, b, slot = i // B, i % B, i % _NBUF
        return pltpu.make_async_copy(
            v_hbm.at[b, h, pl.ds(vs, Sk - vs)],
            vbuf.at[slot, pl.ds(vs, Sk - vs)],
            sems.at[3, slot],
        )

    def start_reads(i):
        for c in early_copies(i):
            c.start()
        late_copy(i).start()

    def start_writes(h):
        for r in range(Sq // _W_ROWS):
            rows = pl.ds(r * _W_ROWS, _W_ROWS)
            pltpu.make_async_copy(
                obuf.at[h, :, rows], o_hbm.at[:, h, rows], osem
            ).start()

    for j in range(_NBUF - 1):
        start_reads(j)

    def body(i, carry):
        slot = i % _NBUF

        @pl.when(i + _NBUF - 1 < n)
        def _():
            start_reads(i + _NBUF - 1)

        @pl.when(i < n - 1)
        def _():
            for c in early_copies(i):
                c.wait()

        late_copy(i).wait()

        @pl.when(i == n - 2)
        def _():
            for c in early_copies(n - 1):
                c.wait()

            def write_head(h, c):
                start_writes(h)
                return c

            jax.lax.fori_loop(0, H - 1, write_head, 0)

        o = _attention_head(qbuf[slot], kbuf[slot], vbuf[slot], scale)
        obuf[i // B, i % B] = o.astype(obuf.dtype)
        return carry

    jax.lax.fori_loop(0, n, body, 0)
    start_writes(H - 1)
    pltpu.make_async_copy(o_hbm, o_hbm, osem).wait()


@jax.jit
def pallas_standalone__mha_softmax__near_ridge_kernel(
    q: jax.Array,
    k: jax.Array,
    v: jax.Array,
):
    B, H, Sq, D = q.shape
    Sk = k.shape[2]
    scale = float(D) ** -0.5
    return pl.pallas_call(
        functools.partial(_kernel, scale=scale),
        in_specs=[pl.BlockSpec(memory_space=pl.ANY)] * 3,
        out_specs=pl.BlockSpec(memory_space=pl.ANY),
        out_shape=jax.ShapeDtypeStruct((B, H, Sq, D), q.dtype),
        scratch_shapes=[
            pltpu.VMEM((_NBUF, Sq, D), q.dtype),
            pltpu.VMEM((_NBUF, Sk, D), k.dtype),
            pltpu.VMEM((_NBUF, Sk, D), v.dtype),
            pltpu.VMEM((H, B, Sq, D), q.dtype),
            pltpu.SemaphoreType.DMA((4, _NBUF)),
            pltpu.SemaphoreType.DMA(()),
        ],
        compiler_params=pltpu.CompilerParams(vmem_limit_bytes=64 * 1024 * 1024),
    )(q, k, v)
```

```python
import functools

import jax
import jax.numpy as jnp
import jax.experimental.pallas as pl
import jax.experimental.pallas.tpu as pltpu

_NBUF = 4
_W_ROWS = 32


def _attention_head(q, k, v, scale):
    s = jax.lax.dot_general(
        q, k, (((1,), (1,)), ((), ())), preferred_element_type=jnp.float32
    )
    m = jnp.max(s, axis=-1, keepdims=True)
    p = jnp.exp((s - m) * scale)
    l = jnp.sum(p, axis=-1, keepdims=True)
    o = jnp.dot(p.astype(v.dtype), v, preferred_element_type=jnp.float32)
    return o / l


def _kernel(q_hbm, k_hbm, v_hbm, o_hbm, qbuf, kbuf, vbuf, obuf, osem, *, scale):
    B, H, Sq, _ = q_hbm.shape
    n = B * H

    def start_writes(h):
        for r in range(Sq // _W_ROWS):
            rows = pl.ds(r * _W_ROWS, _W_ROWS)
            pltpu.make_async_copy(
                obuf.at[h, :, rows], o_hbm.at[:, h, rows], osem
            ).start()

    def stream(sems):
        def read(j, i):
            src, dst = ((q_hbm, qbuf), (k_hbm, kbuf), (v_hbm, vbuf))[j]
            slot = i % _NBUF
            return pltpu.make_async_copy(
                src.at[i % B, i // B], dst.at[slot], sems.at[j, slot]
            )

        def start_reads(i):
            for j in range(3):
                read(j, i).start()

        def wait_qk(i):
            read(0, i).wait()
            read(1, i).wait()

        for i in range(_NBUF - 1):
            start_reads(i)

        def body(i, carry):
            @pl.when(i + _NBUF - 1 < n)
            def _():
                start_reads(i + _NBUF - 1)

            @pl.when(i < n - 1)
            def _():
                wait_qk(i)

            read(2, i).wait()

            @pl.when(i == n - 2)
            def _():
                wait_qk(n - 1)

                def write_head(h, c):
                    start_writes(h)
                    return c

                jax.lax.fori_loop(0, H - 1, write_head, 0)

            slot = i % _NBUF
            o = _attention_head(qbuf[slot], kbuf[slot], vbuf[slot], scale)
            obuf[i // B, i % B] = o.astype(obuf.dtype)
            return carry

        jax.lax.fori_loop(0, n, body, 0)
        start_writes(H - 1)

    pl.run_scoped(stream, pltpu.SemaphoreType.DMA((3, _NBUF)))
    pltpu.make_async_copy(o_hbm, o_hbm, osem).wait()


@jax.jit
def pallas_standalone__mha_softmax__near_ridge_kernel(
    q: jax.Array,
    k: jax.Array,
    v: jax.Array,
):
    B, H, Sq, D = q.shape
    Sk = k.shape[2]
    assert B >= 2 and Sq % _W_ROWS == 0 and B * H >= _NBUF
    scale = float(D) ** -0.5
    return pl.pallas_call(
        functools.partial(_kernel, scale=scale),
        in_specs=[pl.BlockSpec(memory_space=pl.ANY)] * 3,
        out_specs=pl.BlockSpec(memory_space=pl.ANY),
        out_shape=jax.ShapeDtypeStruct((B, H, Sq, D), q.dtype),
        scratch_shapes=[
            pltpu.VMEM((_NBUF, Sq, D), q.dtype),
            pltpu.VMEM((_NBUF, Sk, D), k.dtype),
            pltpu.VMEM((_NBUF, Sk, D), v.dtype),
            pltpu.VMEM((H, B, Sq, D), q.dtype),
            pltpu.SemaphoreType.DMA(()),
        ],
        compiler_params=pltpu.CompilerParams(vmem_limit_bytes=64 * 1024 * 1024),
    )(q, k, v)
```
